```python
import jax
import jax.numpy as jnp

def _softmax(x, axis=-1):
    return jax.nn.softmax(x, axis=axis)
def _gelu(x):
    return jax.nn.gelu(x, approximate=True)
def _silu(x):
    return jax.nn.silu(x)
def _sigmoid(x):
    return jax.nn.sigmoid(x)
def _layernorm(x, axis=-1, eps=1e-5):
    m = jnp.mean(x, axis=axis, keepdims=True)
    v = jnp.var(x, axis=axis, keepdims=True)
    return (x - m) / jnp.sqrt(v + eps)
def _scatter_add(tgt, idx, src, axis=0):
    return tgt.at[idx].add(src)
def _segment_sum(src, seg, n):
    return jax.ops.segment_sum(src, seg, n)
class _Rng:
    def __init__(self, key):
        self._k = key
    def _next(self):
        self._k, sub = jax.random.split(self._k)
        return sub
    def normal(self, shape):
        return jax.random.normal(self._next(), shape, dtype=jnp.bfloat16)
    def randint(self, lo, hi, shape):
        return jax.random.randint(self._next(), shape, lo, hi, dtype=jnp.int32)
    def uniform(self, shape, lo=0.0, hi=1.0):
        return jax.random.uniform(self._next(), shape, jnp.bfloat16, lo, hi)
    def permutation(self, n):
        return jax.random.permutation(self._next(), n)


kernel_name = 'sequential_preLN__sliding_block_cached__mixer_s_mlp__decode'

def setup_inputs():
    _rng = _Rng(jax.random.key(int.from_bytes(__import__("os").urandom(4), "little")))
    _w = (lambda a: (lambda t: t.astype(jnp.bfloat16) if jnp.issubdtype(t.dtype, jnp.floating) else t)(jnp.asarray(a)))
    def _A_setup():
        B, Sq, D = 1, 1, 640
        Hq, Hkv, Sk, Dh = 32, 32, 32768, 192
        assert Hq % Hkv == 0, (Hq, Hkv)
        return {
            "x": _w((lambda *s: _rng.normal(s) * 0.05)(B, Sq, D)),
            "k_cache": _w((lambda *s: _rng.normal(s) * 0.05)(B, Hkv, Sk, Dh)),
            "v_cache": _w((lambda *s: _rng.normal(s) * 0.05)(B, Hkv, Sk, Dh)),
            "wq": _w((lambda *s: _rng.normal(s) * 0.05)(D, Hq * Dh) * (D ** -0.5)),
            "wo": _w((lambda *s: _rng.normal(s) * 0.05)(Hq * Dh, D) * ((Hq * Dh) ** -0.5)),
        }
    _A_in = _A_setup()

    def _B_setup():
        B, S, D, F = 1, 1, 640, 1536
        return {
            "x":  _w((lambda *s: _rng.normal(s) * 0.05)(B, S, D)),
            "w1": _w((lambda *s: _rng.normal(s) * 0.05)(D, D) * (D ** -0.5)),
            "w2": _w((lambda *s: _rng.normal(s) * 0.05)(D, D) * (D ** -0.5)),
            "w3": _w((lambda *s: _rng.normal(s) * 0.05)(D, F) * (D ** -0.5)),
            "w4": _w((lambda *s: _rng.normal(s) * 0.05)(F, D) * (F ** -0.5)),
        }
    _B_in = _B_setup()

    return {
        "A_x": _A_in["x"],
        "A_k_cache": _A_in["k_cache"],
        "A_v_cache": _A_in["v_cache"],
        "A_wq": _A_in["wq"],
        "A_wo": _A_in["wo"],
        "B_x": _B_in["x"],
        "B_w1": _B_in["w1"],
        "B_w2": _B_in["w2"],
        "B_w3": _B_in["w3"],
        "B_w4": _B_in["w4"],
    }

def reference(A_x, A_k_cache, A_v_cache, A_wq, A_wo, B_x, B_w1, B_w2, B_w3, B_w4):
    def _A_ref(x, k_cache, v_cache, wq, wo):
        B, Sq, D = x.shape
        Hq, Dh = 32, 192
        Hkv, Sk = k_cache.shape[1], k_cache.shape[2]
        W = min(4096, max(256, Sk // 4))
        rep = Hq // Hkv
        q = (lambda x, *d: x.transpose(*d))((x @ wq).reshape(B, Sq, Hq, Dh), 0, 2, 1, 3)
        k = jnp.repeat(k_cache[:, :, Sk - W:, :], rep, axis=1)
        v = jnp.repeat(v_cache[:, :, Sk - W:, :], rep, axis=1)
        scores = jnp.einsum("bhqd,bhkd->bhqk", q, k) * (Dh ** -0.5)
        p = _softmax(scores, axis=-1)
        o = jnp.einsum("bhqk,bhkd->bhqd", p, v)
        return (lambda x, *d: x.transpose(*d))(o, 0, 2, 1, 3).reshape(B, Sq, Hq * Dh) @ wo

    def _B_ref(x, w1, w2, w3, w4):
        B, S, D = x.shape
        h = _gelu(_layernorm(x, axis=-1) @ w1)
        c = D // 4
        g0 = jnp.pad(h[:, :, 0*c:1*c], ((0, 0), (1, 0), (0, 0)))[:, :S, :]
        g1 = jnp.pad(h[:, :, 1*c:2*c], ((0, 0), (0, 1), (0, 0)))[:, 1:, :]
        g2 = jnp.pad(h[:, :, 2*c:3*c], ((0, 0), (2, 0), (0, 0)))[:, :S, :]
        g3 = jnp.pad(h[:, :, 3*c:   ], ((0, 0), (0, 2), (0, 0)))[:, 2:, :]
        hs = jnp.concatenate([g0, g1, g2, g3], axis=-1) @ w2
        x1 = x + hs
        h2 = _gelu(_layernorm(x1, axis=-1) @ w3) @ w4
        return x1 + h2

    x = A_x
    h = x + _A_ref(_layernorm(x, axis=-1), A_k_cache, A_v_cache, A_wq, A_wo)
    h2 = h + _B_ref(_layernorm(h, axis=-1), B_w1, B_w2, B_w3, B_w4)
    return h2
```

```python
import functools
import jax
import jax.numpy as jnp
from jax import lax
from jax.experimental import pallas as pl
from jax.experimental.pallas import tpu as pltpu

D = 640
H = 32
DH = 192
SK = 32768
W = 4096
F = 1536
EPS = 1e-5
SCALE = DH ** -0.5


def _ln(x):
    m = jnp.mean(x, axis=-1, keepdims=True)
    c = x - m
    v = jnp.mean(c * c, axis=-1, keepdims=True)
    return c / jnp.sqrt(v + EPS)


def build(KR=96, KC=256, NS=2, LA=5, dma=True, compute=True, bounds=False, extra=0):
    NQ = 16
    QC = 2 * DH
    NO = 16
    N3 = 6; C3 = F // N3
    N4 = 6; R4 = F // (2 * N4)
    SW = W // NS
    UD = (DH // KR) * (SW // KC)
    PER = 2 * NS
    assert LA <= PER + NS

    def kernel(x_hbm, k_hbm, v_hbm, wq_hbm, wo_hbm, w3_hbm, w4_hbm, o_ref,
               xb, wqb, kb, vb, wob, w3b, w4b, qs, os_,
               sx, sq, sk, sv, so, s3, s4):
        def mk(src, dst, sem, p):
            def go():
                if dma:
                    pltpu.make_async_copy(src, dst, sem).start(priority=p)
            return go
        def wt(dst, sem):
            if dma:
                pltpu.make_async_copy(dst, dst, sem).wait()

        def kv_descs(h, u):
            kv, s = divmod(u, NS)
            hbm, buf, sem = (k_hbm, kb, sk) if kv == 0 else (v_hbm, vb, sv)
            slot = h % 2
            nr = DH // KR
            l = []
            for ic in range(SW // KC):
                for ir in range(nr // 2):
                    for p in range(2):
                        r0 = (ir + p * (nr // 2)) * KR
                        l.append(mk(hbm.at[h, pl.ds(r0, KR), pl.ds(SK - W + s * SW + ic * KC, KC)],
                                    buf.at[slot, s, pl.ds(r0, KR), pl.ds(ic * KC, KC)], sem.at[slot, s], p))
            return l

        def wq_descs(g):
            return [mk(wq_hbm.at[pl.ds((ir + 5 * p) * 64, 64), pl.ds(g * QC, QC)],
                       wqb.at[g, pl.ds((ir + 5 * p) * 64, 64), :], sq.at[g], p)
                    for ir in range(5) for p in range(2)]

        def wo_descs(j):
            return [mk(wo_hbm.at[pl.ds((j + 16 * p) * DH + ir * 32, 32), :],
                       wob.at[j, p, pl.ds(ir * 32, 32), :], so.at[j], p)
                    for ir in range(6) for p in range(2)]

        def w3_descs(j):
            return [mk(w3_hbm.at[pl.ds((ir + 4 * p) * 80, 80), pl.ds(j * C3, C3)],
                       w3b.at[j, pl.ds((ir + 4 * p) * 80, 80), :], s3.at[j], p)
                    for ir in range(4) for p in range(2)]

        def w4_descs(j):
            return [mk(w4_hbm.at[pl.ds((j + N4 * p) * R4 + ir * 32, 32), :],
                       w4b.at[j, p, pl.ds(ir * 32, 32), :], s4.at[j], p)
                    for ir in range(4) for p in range(2)]

        class Pump:
            def __init__(self, l):
                self.l = l; self.i = 0
            def issue(self, n):
                for d in self.l[self.i:self.i + n]:
                    d()
                self.i = min(len(self.l), self.i + n)

        QD = LA * UD
        head_l = [mk(x_hbm, xb, sx, 0)]
        for g in range(NQ):
            head_l += wq_descs(g)
        for gu in range(LA):
            head_l += kv_descs(gu // PER, gu % PER)
        p1 = Pump(head_l)
        p1.issue(QD + 1)

        wt(xb, sx)
        x = xb[0].astype(jnp.float32)
        xn = _ln(x)
        xn8 = jnp.broadcast_to(xn, (8, D)).astype(jnp.bfloat16)
        for g in range(NQ):
            wt(wqb.at[g], sq.at[g])
            p1.issue(10)
            if compute:
                q2 = jnp.dot(xn8, wqb[g], preferred_element_type=jnp.float32)
                qs[2 * g] = q2[:, :DH]
                qs[2 * g + 1] = q2[:, DH:]
        assert p1.i == len(head_l)

        tail_l = []
        for j in range(NO):
            tail_l += wo_descs(j)
        for j in range(N3):
            tail_l += w3_descs(j)
        for j in range(N4):
            tail_l += w4_descs(j)
        p3 = Pump(tail_l)

        def head(h, carry):
            slot = h % 2
            def site(u):
                dh, uu = divmod(u + LA, PER)
                @pl.when(h + dh < H)
                def _():
                    for d in kv_descs(h + dh, uu):
                        d()
                for hh in range(H - dh, H):
                    g = hh * PER + u + LA - H * PER
                    @pl.when(h == hh)
                    def _():
                        for d in tail_l[g * UD:(g + 1) * UD]:
                            d()
            q = qs[h].astype(jnp.bfloat16)
            ss = []
            for s in range(NS):
                wt(kb.at[slot, s], sk.at[slot, s])
                site(s)
                if compute:
                    ss.append(jnp.dot(q, kb[slot, s], preferred_element_type=jnp.float32) * SCALE)
            if compute:
                s_ = jnp.concatenate(ss, axis=1)
                m = jnp.max(s_, axis=1, keepdims=True)
                p = jnp.exp(s_ - m)
                l = jnp.sum(p, axis=1, keepdims=True)
                pb = p.astype(jnp.bfloat16)
                o = jnp.zeros((8, DH), jnp.float32)
            for s in range(NS):
                wt(vb.at[slot, s], sv.at[slot, s])
                site(NS + s)
                if compute:
                    o = o + lax.dot_general(pb[:, s * SW:(s + 1) * SW], vb[slot, s], (((1,), (1,)), ((), ())),
                                            preferred_element_type=jnp.float32)
            if compute:
                os_[h] = o / l
            return carry

        lax.fori_loop(0, H, head, 0)
        p3.i = QD

        acc = jnp.zeros((8, D), jnp.float32)
        for j in range(NO):
            wt(wob.at[j], so.at[j])
            p3.issue(12)
            if compute:
                for p in range(2):
                    acc = acc + jnp.dot(os_[j + 16 * p].astype(jnp.bfloat16), wob[j, p],
                                        preferred_element_type=jnp.float32)
        attn = acc[0:1]
        hres = x + attn
        x1 = _ln(hres)
        y = _ln(x1)
        y8 = jnp.broadcast_to(y, (8, D)).astype(jnp.bfloat16)
        mids = []
        for j in range(N3):
            wt(w3b.at[j], s3.at[j])
            p3.issue(8)
            if compute:
                t = jnp.dot(y8, w3b[j], preferred_element_type=jnp.float32)
                mids.append(jax.nn.gelu(t, approximate=True).astype(jnp.bfloat16))
        if compute:
            mid = jnp.concatenate(mids, axis=1)
        assert p3.i == len(tail_l)
        acc2 = jnp.zeros((8, D), jnp.float32)
        for j in range(N4):
            wt(w4b.at[j], s4.at[j])
            if compute:
                for p in range(2):
                    jj = j + N4 * p
                    acc2 = acc2 + jnp.dot(mid[:, jj * R4:(jj + 1) * R4], w4b[j, p],
                                          preferred_element_type=jnp.float32)
        out = hres + (x1 + acc2[0:1])
        o_ref[0] = out.astype(o_ref.dtype)

    @jax.jit
    def f(A_x, A_k_cache, A_v_cache, A_wq, A_wo, B_x, B_w1, B_w2, B_w3, B_w4):
        kt = jnp.swapaxes(A_k_cache, 2, 3).reshape(H, DH, SK)
        vt = jnp.swapaxes(A_v_cache, 2, 3).reshape(H, DH, SK)
        bf = jnp.bfloat16
        return pl.pallas_call(
            kernel,
            in_specs=[pl.BlockSpec(memory_space=pl.ANY)] * 7,
            out_specs=pl.BlockSpec(memory_space=pltpu.VMEM),
            out_shape=jax.ShapeDtypeStruct((1, 1, D), bf),
            scratch_shapes=[
                pltpu.VMEM((1, 1, D), bf),
                pltpu.VMEM((NQ, D, QC), bf),
                pltpu.VMEM((2, NS, DH, SW), bf),
                pltpu.VMEM((2, NS, DH, SW), bf),
                pltpu.VMEM((NO, 2, DH, D), bf),
                pltpu.VMEM((N3, D, C3), bf),
                pltpu.VMEM((N4, 2, R4, D), bf),
                pltpu.VMEM((H, 8, DH), jnp.float32),
                pltpu.VMEM((H, 8, DH), jnp.float32),
                pltpu.SemaphoreType.DMA(()),
                pltpu.SemaphoreType.DMA((NQ,)),
                pltpu.SemaphoreType.DMA((2, NS)),
                pltpu.SemaphoreType.DMA((2, NS)),
                pltpu.SemaphoreType.DMA((NO,)),
                pltpu.SemaphoreType.DMA((N3,)),
                pltpu.SemaphoreType.DMA((N4,)),
            ],
            compiler_params=pltpu.CompilerParams(vmem_limit_bytes=100 * 1024 * 1024,
                                                 disable_bounds_checks=not bounds),
        )(A_x, kt, vt, A_wq, A_wo, B_w3, B_w4)
    return f


_F = build(LA=6)


def pallas_sequential_preLN__sliding_block_cached__mixer_s_mlp__decode_kernel(
        A_x, A_k_cache, A_v_cache, A_wq, A_wo, B_x, B_w1, B_w2, B_w3, B_w4):
    return _F(A_x, A_k_cache, A_v_cache, A_wq, A_wo, B_x, B_w1, B_w2, B_w3, B_w4)
```

```python
import functools
import jax
import jax.numpy as jnp
from jax import lax
from jax.experimental import pallas as pl
from jax.experimental.pallas import tpu as pltpu

D = 640
H = 32
DH = 192
SK = 32768
W = 4096
F = 1536
EPS = 1e-5
SCALE = DH ** -0.5


def _ln(x):
    m = jnp.mean(x, axis=-1, keepdims=True)
    c = x - m
    v = jnp.mean(c * c, axis=-1, keepdims=True)
    return c / jnp.sqrt(v + EPS)


def build(KR=32, KC=512, NS=2, LA=4, QD=96, dma=True, compute=True, bounds=False,
          R4=128, D4=16, TV=4, outmode="tiles"):
    QC = 2 * DH
    GQ, RQ = 10, 64
    GO, RO = 8, 768
    NO = 16
    G3, R3 = 8, 80
    N3 = 5
    N4 = F // (2 * R4)
    NM = N4 - 1 if TV else N4
    RV = R4 // TV if TV else 0
    SW = W // NS
    UD = (DH // KR) * (SW // KC)
    PER = 2 * NS
    assert LA <= 2 * PER - 1

    def kernel(x_hbm, k_hbm, v_hbm, wq_hbm, wo_hbm, w3_hbm, w4_hbm, o_ref,
               xb, wqb, kb, vb, wob, w3b, w4b, qs, os_,
               sx, sq, sk, sv, so, s3, s4):
        def mk(src, dst, sem, p):
            def go():
                if dma:
                    pltpu.make_async_copy(src, dst, sem).start(priority=p)
            return go
        def wt(dst, sem):
            if dma:
                pltpu.make_async_copy(dst, dst, sem).wait()

        def kv_descs(h, u):
            kv, s = divmod(u, NS)
            hbm, buf, sem = (k_hbm, kb, sk) if kv == 0 else (v_hbm, vb, sv)
            slot = h % 2
            nr = DH // KR
            l = []
            for ic in range(SW // KC):
                for ir in range(nr // 2):
                    for p in range(2):
                        r0 = (ir + p * (nr // 2)) * KR
                        l.append(mk(hbm.at[h, pl.ds(r0, KR), pl.ds(SK - W + s * SW + ic * KC, KC)],
                                    buf.at[slot, s, pl.ds(r0, KR), pl.ds(ic * KC, KC)], sem.at[slot, s], p))
            return l

        def same(hbm, buf, idx, sem, p):
            return mk(hbm.at[idx], buf.at[idx], sem, p)

        def wq_descs(r):
            return [same(wq_hbm, wqb, (pl.ds(5 * p, 5), pl.ds(8 * r, 8), pl.ds(c * 512, 512)), sq.at[r], p)
                    for c in range(H * DH // 512) for p in range(2)]

        def wo_descs(j):
            return [same(wo_hbm, wob, (pl.ds(4 * p + 2 * g, 2), pl.ds(48 * j + 16 * r, 16), slice(None)), so.at[j], p)
                    for r in range(3) for g in range(2) for p in range(2)]

        def w3_descs(j):
            return [same(w3_hbm, w3b, (pl.ds(4 * p, 4), pl.ds(16 * j + 8 * r, 8), pl.ds(c * 512, 512)), s3.at[j], p)
                    for r in range(2) for c in range(3) for p in range(2)]

        def w4_descs(j):
            return [mk(w4_hbm.at[pl.ds((j + N4 * p) * R4 + ir * D4, D4), :],
                       w4b.at[j, p, pl.ds(ir * D4, D4), :], s4.at[j], p)
                    for ir in range(R4 // D4) for p in range(2)]

        def w4v_descs(t):
            j = N4 - 1
            dd = min(D4, RV)
            return [mk(w4_hbm.at[pl.ds((j + N4 * p) * R4 + t * RV + ir * dd, dd), :],
                       w4b.at[j, p, pl.ds(t * RV + ir * dd, dd), :], s4.at[NM + t], p)
                    for ir in range(RV // dd) for p in range(2)]

        class Pump:
            def __init__(self, l):
                self.l = l; self.i = 0
            def issue(self, n):
                for d in self.l[self.i:self.i + n]:
                    d()
                self.i = min(len(self.l), self.i + n)

        head_l = [mk(x_hbm, xb, sx, 0)]
        for r in range(RQ // 8):
            head_l += wq_descs(r)
        for gu in range(LA):
            head_l += kv_descs(gu // PER, gu % PER)
        p1 = Pump(head_l)
        p1.issue(len(head_l) - 24 * 8)

        wt(xb, sx)
        x = xb[0].astype(jnp.float32)
        xn = _ln(x)
        xn8 = jnp.broadcast_to(xn, (8, D)).astype(jnp.bfloat16)
        for r in range(RQ // 8):
            wt(wqb.at[:, pl.ds(8 * r, 8), :], sq.at[r])
            p1.issue(24)
        assert p1.i == len(head_l)

        tail_u = [wo_descs(j) for j in range(NO)] + [w3_descs(j) for j in range(N3)] + [w4_descs(j) for j in range(NM)] + [w4v_descs(t) for t in range(TV)]
        tail_l = [d for u in tail_u for d in u]
        p3 = Pump(tail_l)
        TS = [QD // LA + (1 if i < QD % LA else 0) for i in range(LA)]
        TO = [sum(TS[:i]) for i in range(LA + 1)]

        def head(h, carry):
            slot = h % 2
            def site(u):
                dh, uu = divmod(u + LA, PER)
                @pl.when(h + dh < H)
                def _():
                    for d in kv_descs(h + dh, uu):
                        d()
                for hh in range(H - dh, H):
                    g = hh * PER + u + LA - H * PER
                    @pl.when(h == hh)
                    def _():
                        for d in tail_l[TO[g]:TO[g + 1]]:
                            d()
            if compute:
                @pl.when(slot == 0)
                def _():
                    c0 = pl.multiple_of((h // 2) * QC, 128)
                    w = wqb[:, :, pl.ds(c0, QC)].reshape(D, QC)
                    q2 = jnp.dot(xn8, w, preferred_element_type=jnp.float32)
                    qs[0] = q2[:, :DH]
                    qs[1] = q2[:, DH:]
                q = qs[slot].astype(jnp.bfloat16)
            ss = []
            for s in range(NS):
                wt(kb.at[slot, s], sk.at[slot, s])
                site(s)
                if compute:
                    ss.append(jnp.dot(q, kb[slot, s], preferred_element_type=jnp.float32) * SCALE)
            if compute:
                s_ = jnp.concatenate(ss, axis=1)
                m = jnp.max(s_, axis=1, keepdims=True)
                p = jnp.exp(s_ - m)
                l = jnp.sum(p, axis=1, keepdims=True)
                pb = p.astype(jnp.bfloat16)
                o = jnp.zeros((8, DH), jnp.float32)
            for s in range(NS):
                wt(vb.at[slot, s], sv.at[slot, s])
                site(NS + s)
                if compute:
                    o = o + lax.dot_general(pb[:, s * SW:(s + 1) * SW], vb[slot, s], (((1,), (1,)), ((), ())),
                                            preferred_element_type=jnp.float32)
            if compute:
                os_[h] = o / l
            return carry

        lax.fori_loop(0, H, head, 0)
        p3.i = QD

        acc = jnp.zeros((8, D), jnp.float32)
        for j in range(NO):
            wt(wob.at[:, pl.ds(48 * j, 48), :], so.at[j])
            p3.issue(len(tail_u[j]))
            if compute and j % 4 == 3:
                i = j // 4
                for g in range(GO):
                    acc = acc + jnp.dot(os_[4 * g + i].astype(jnp.bfloat16), wob[g, i * DH:(i + 1) * DH, :],
                                        preferred_element_type=jnp.float32)
        attn = acc[0:1]
        hres = x + attn
        x1 = _ln(hres)
        y = _ln(x1)
        y8 = jnp.broadcast_to(y, (8, D)).astype(jnp.bfloat16)
        for j in range(N3):
            wt(w3b.at[:, pl.ds(16 * j, 16), :], s3.at[j])
            p3.issue(len(tail_u[NO + j]))
        if compute:
            t = jnp.dot(y8, w3b[...].reshape(D, F), preferred_element_type=jnp.float32)
            mid = jax.nn.gelu(t, approximate=True).astype(jnp.bfloat16)
        acc2 = jnp.broadcast_to(hres + x1, (8, D))
        if compute and TV:
            mf = mid.astype(jnp.float32)
            mcol = [jnp.broadcast_to(mf[0:1, (N4 - 1 + N4 * p) * R4:(N4 + N4 * p) * R4], (128, R4)).T for p in range(2)]
        for j in range(NM):
            wt(w4b.at[j], s4.at[j])
            p3.issue(len(tail_u[NO + N3 + j]))
            if compute:
                for p in range(2):
                    jj = j + N4 * p
                    acc2 = acc2 + jnp.dot(mid[:, jj * R4:(jj + 1) * R4], w4b[j, p],
                                          preferred_element_type=jnp.float32)
        assert p3.i == len(tail_l)
        accv = None
        for t in range(TV):
            wt(w4b.at[N4 - 1, :, pl.ds(t * RV, RV), :], s4.at[NM + t])
            if compute:
                for p in range(2):
                    w = w4b[N4 - 1, p, t * RV:(t + 1) * RV, :].astype(jnp.float32)
                    mc = mcol[p][t * RV:(t + 1) * RV]
                    prod = w * jnp.concatenate([mc] * (D // 128), axis=1)
                    part = jnp.sum(prod.reshape(RV // 8, 8, D), axis=0)
                    accv = part if accv is None else accv + part
        out = acc2[0:1]
        if accv is not None:
            out = out + jnp.sum(accv, axis=0, keepdims=True)
        if outmode == "tiles":
            for j in range(D // 128):
                o_ref[0, :, j * 128:(j + 1) * 128] = out[:, j * 128:(j + 1) * 128].astype(o_ref.dtype)
        else:
            o_ref[0] = out.astype(o_ref.dtype)

    @jax.jit
    def f(A_x, A_k_cache, A_v_cache, A_wq, A_wo, B_x, B_w1, B_w2, B_w3, B_w4):
        kt = jnp.swapaxes(A_k_cache, 2, 3).reshape(H, DH, SK)
        vt = jnp.swapaxes(A_v_cache, 2, 3).reshape(H, DH, SK)
        bf = jnp.bfloat16
        return pl.pallas_call(
            kernel,
            in_specs=[pl.BlockSpec(memory_space=pl.ANY)] * 7,
            out_specs=pl.BlockSpec(memory_space=pltpu.VMEM),
            out_shape=jax.ShapeDtypeStruct((1, 1, D), bf),
            scratch_shapes=[
                pltpu.VMEM((1, 1, D), bf),
                pltpu.VMEM((GQ, RQ, H * DH), bf),
                pltpu.VMEM((2, NS, DH, SW), bf),
                pltpu.VMEM((2, NS, DH, SW), bf),
                pltpu.VMEM((GO, RO, D), bf),
                pltpu.VMEM((G3, R3, F), bf),
                pltpu.VMEM((N4, 2, R4, D), bf),
                pltpu.VMEM((2, 8, DH), jnp.float32),
                pltpu.VMEM((H, 8, DH), jnp.float32),
                pltpu.SemaphoreType.DMA(()),
                pltpu.SemaphoreType.DMA((RQ // 8,)),
                pltpu.SemaphoreType.DMA((2, NS)),
                pltpu.SemaphoreType.DMA((2, NS)),
                pltpu.SemaphoreType.DMA((NO,)),
                pltpu.SemaphoreType.DMA((N3,)),
                pltpu.SemaphoreType.DMA((NM + TV,)),
            ],
            compiler_params=pltpu.CompilerParams(vmem_limit_bytes=100 * 1024 * 1024,
                                                 disable_bounds_checks=not bounds,
                                                 disable_semaphore_checks=not bounds),
        )(A_x, kt, vt, A_wq.reshape(GQ, RQ, H * DH), A_wo.reshape(GO, RO, D), B_w3.reshape(G3, R3, F), B_w4)
    return f


_F = build()


def pallas_sequential_preLN__sliding_block_cached__mixer_s_mlp__decode_kernel(
        A_x, A_k_cache, A_v_cache, A_wq, A_wo, B_x, B_w1, B_w2, B_w3, B_w4):
    return _F(A_x, A_k_cache, A_v_cache, A_wq, A_wo, B_x, B_w1, B_w2, B_w3, B_w4)
```

```python
import jax
import jax.numpy as jnp
from jax import lax
from jax.experimental import pallas as pl
from jax.experimental.pallas import tpu as pltpu

D = 640
H = 32
DH = 192
F = 1536
EPS = 1e-5
SCALE = DH ** -0.5

KR, KC, KFIRST = 32, 512, 256
KSPLIT = 5
LA = 5
QD = 96
GQ, RQ, CQ = 10, 64, 640
GO, RO, NO = 8, 768, 16
G3, R3, N3 = 8, 80, 5
R4, D4 = 128, 16
N4 = F // (2 * R4)
TV = 4
RV = R4 // TV
QC = 2 * DH


def _ln(x):
    m = jnp.mean(x, axis=-1, keepdims=True)
    c = x - m
    v = jnp.mean(c * c, axis=-1, keepdims=True)
    return c / jnp.sqrt(v + EPS)


def _splits(total, c, first=None):
    b = [0] if first is None else [0, first]
    while b[-1] + c < total:
        b.append(b[-1] + c)
    b.append(total)
    return [(b[i], b[i + 1] - b[i]) for i in range(len(b) - 1)]


def _kv_groups(w):
    cs = _splits(w, KC, KFIRST)
    groups = []
    for kv in range(2):
        for part in (cs[:KSPLIT], cs[KSPLIT:]):
            blocks = []
            for c0, cw in part:
                r = KR if cw == KC else DH // 2
                for r0 in range(0, DH // 2, r):
                    for p in range(2):
                        blocks.append((r0 + p * (DH // 2), r, c0, cw, p))
            groups.append((kv, part[0][0], part[-1][0] + part[-1][1], blocks))
    return groups


def _make_kernel(sk, w):
    groups = _kv_groups(w)
    per = len(groups)
    nt = (((1,), (1,)), ((), ()))

    def kernel(x_hbm, k_hbm, v_hbm, wq_hbm, wo_hbm, w3_hbm, w4_hbm, o_ref,
               xb, wqb, kvb, wob, w3b, w4b, qs, ob,
               sx, sq, skv, so, s3, s4):

        def start(copies):
            for src, dst, sem, p in copies:
                pltpu.make_async_copy(src, dst, sem).start(priority=p)

        def wait(dst, sem):
            pltpu.make_async_copy(dst, dst, sem).wait()

        def same(hbm, buf, idx, sem, p):
            return (hbm.at[idx], buf.at[idx], sem, p)

        def kv_copies(h, u):
            kv = groups[u][0]
            slot = h % 2
            return [((k_hbm, v_hbm)[kv].at[h, pl.ds(r0, nr), pl.ds(sk - w + c0, nc)],
                     kvb.at[slot, kv, pl.ds(r0, nr), pl.ds(c0, nc)], skv.at[slot, u], p)
                    for (r0, nr, c0, nc, p) in groups[u][3]]

        def wq_copies(r):
            return [same(wq_hbm, wqb, (pl.ds(p * (GQ // 2), GQ // 2), pl.ds(8 * r, 8), pl.ds(c0, cw)), sq.at[r], p)
                    for (c0, cw) in _splits(H * DH, CQ) for p in range(2)]

        def wo_copies(j):
            return [same(wo_hbm, wob, (pl.ds(4 * p + 2 * g, 2), pl.ds(48 * j + 16 * r, 16), slice(None)), so.at[j], p)
                    for r in range(3) for g in range(2) for p in range(2)]

        def w3_copies(j):
            return [same(w3_hbm, w3b, (pl.ds(4 * p, 4), pl.ds(16 * j + 8 * r, 8), pl.ds(c * 512, 512)), s3.at[j], p)
                    for r in range(2) for c in range(3) for p in range(2)]

        def w4_copies(j, r0, rows, sem):
            return [(w4_hbm.at[pl.ds((j + N4 * p) * R4 + r, D4), :], w4b.at[j, p, pl.ds(r, D4), :], sem, p)
                    for r in range(r0, r0 + rows, D4) for p in range(2)]

        nq = len(wq_copies(0))
        first = [(x_hbm, xb, sx, 0)]
        for r in range(RQ // 8):
            first += wq_copies(r)
        for g in range(LA):
            first += kv_copies(g // per, g % per)
        pos = len(first) - nq * (RQ // 8)
        start(first[:pos])

        wait(xb, sx)
        x = xb[0].astype(jnp.float32)
        xn8 = jnp.broadcast_to(_ln(x), (8, D)).astype(jnp.bfloat16)
        for r in range(RQ // 8):
            wait(wqb.at[:, pl.ds(8 * r, 8), :], sq.at[r])
            start(first[pos:pos + nq])
            pos += nq

        last_groups = ([wo_copies(j) for j in range(NO)] + [w3_copies(j) for j in range(N3)]
                       + [w4_copies(j, 0, R4, s4.at[j]) for j in range(N4 - 1)]
                       + [w4_copies(N4 - 1, t * RV, RV, s4.at[N4 - 1 + t]) for t in range(TV)])
        last = [c for g in last_groups for c in g]
        cut = [(QD * i) // LA for i in range(LA + 1)]

        def head(h, carry):
            slot = h % 2

            @pl.when(slot == 0)
            def _():
                c0 = pl.multiple_of((h // 2) * QC, 128)
                wq2 = wqb[:, :, pl.ds(c0, QC)].reshape(D, QC)
                q2 = jnp.dot(xn8, wq2, preferred_element_type=jnp.float32)
                qs[0] = q2[:, :DH]
                qs[1] = q2[:, DH:]

            q = qs[slot].astype(jnp.bfloat16)

            def arrive(u):
                kv, lo, hi, _ = groups[u]
                wait(kvb.at[slot, kv, :, pl.ds(lo, hi - lo)], skv.at[slot, u])
                dh, un = divmod(u + LA, per)

                @pl.when(h + dh < H)
                def _():
                    start(kv_copies(h + dh, un))

                for hh in range(H - dh, H):
                    g = (hh - H) * per + u + LA

                    @pl.when(h == hh)
                    def _():
                        start(last[cut[g]:cut[g + 1]])
                return lo, hi

            parts = []
            for u in range(per // 2):
                lo, hi = arrive(u)
                parts.append(jnp.dot(q, kvb[slot, 0, :, lo:hi], preferred_element_type=jnp.float32) * SCALE)
            s = jnp.concatenate(parts, axis=1)
            p = jnp.exp(s - jnp.max(s, axis=1, keepdims=True))
            l = jnp.sum(p, axis=1, keepdims=True)
            pb = p.astype(jnp.bfloat16)
            o = jnp.zeros((8, DH), jnp.float32)
            for u in range(per // 2, per):
                lo, hi = arrive(u)
                o = o + lax.dot_general(pb[:, lo:hi], kvb[slot, 1, :, lo:hi], nt,
                                        preferred_element_type=jnp.float32)
            ob[h] = o / l
            return carry

        lax.fori_loop(0, H, head, 0)

        state = {"pos": QD, "g": 0}

        def arrive_last(dst, sem):
            wait(dst, sem)
            n = len(last_groups[state["g"]])
            start(last[state["pos"]:state["pos"] + n])
            state["pos"] += n
            state["g"] += 1

        acc = jnp.zeros((8, D), jnp.float32)
        for j in range(NO):
            arrive_last(wob.at[:, pl.ds(48 * j, 48), :], so.at[j])
            if j % 4 == 3:
                i = j // 4
                for g in range(GO):
                    acc = acc + jnp.dot(ob[4 * g + i].astype(jnp.bfloat16), wob[g, i * DH:(i + 1) * DH, :],
                                        preferred_element_type=jnp.float32)
        hres = x + acc[0:1]
        x1 = _ln(hres)
        y8 = jnp.broadcast_to(_ln(x1), (8, D)).astype(jnp.bfloat16)

        for j in range(N3):
            arrive_last(w3b.at[:, pl.ds(16 * j, 16), :], s3.at[j])
        t = jnp.dot(y8, w3b[...].reshape(D, F), preferred_element_type=jnp.float32)
        mid = jax.nn.gelu(t, approximate=True).astype(jnp.bfloat16)
        mf = mid.astype(jnp.float32)
        mcol = [jnp.broadcast_to(mf[0:1, (N4 - 1 + N4 * p) * R4:(N4 + N4 * p) * R4], (128, R4)).T
                for p in range(2)]
        acc = jnp.broadcast_to(hres + x1, (8, D))
        for j in range(N4 - 1):
            arrive_last(w4b.at[j], s4.at[j])
            for p in range(2):
                jj = j + N4 * p
                acc = acc + jnp.dot(mid[:, jj * R4:(jj + 1) * R4], w4b[j, p],
                                    preferred_element_type=jnp.float32)
        assert state["pos"] >= len(last)
        accv = jnp.zeros((8, D), jnp.float32)
        for t in range(TV):
            wait(w4b.at[N4 - 1, :, pl.ds(t * RV, RV), :], s4.at[N4 - 1 + t])
            for p in range(2):
                wv = w4b[N4 - 1, p, t * RV:(t + 1) * RV, :].astype(jnp.float32)
                mc = mcol[p][t * RV:(t + 1) * RV]
                prod = wv * jnp.concatenate([mc] * (D // 128), axis=1)
                accv = accv + jnp.sum(prod.reshape(RV // 8, 8, D), axis=0)
        out = acc[0:1] + jnp.sum(accv, axis=0, keepdims=True)
        o_ref[0] = out.astype(o_ref.dtype)

    return kernel, per


@jax.jit
def pallas_sequential_preLN__sliding_block_cached__mixer_s_mlp__decode_kernel(
    A_x: jax.Array,
    A_k_cache: jax.Array,
    A_v_cache: jax.Array,
    A_wq: jax.Array,
    A_wo: jax.Array,
    B_x: jax.Array,
    B_w1: jax.Array,
    B_w2: jax.Array,
    B_w3: jax.Array,
    B_w4: jax.Array,
):
    del B_x, B_w1, B_w2
    assert A_x.shape == (1, 1, D) and A_k_cache.shape[:2] == (1, H) and A_k_cache.shape[3] == DH
    sk = A_k_cache.shape[2]
    w = min(4096, max(256, sk // 4))
    kt = jnp.swapaxes(A_k_cache, 2, 3).reshape(H, DH, sk)
    vt = jnp.swapaxes(A_v_cache, 2, 3).reshape(H, DH, sk)
    kernel, per = _make_kernel(sk, w)
    bf = jnp.bfloat16
    dma = pltpu.SemaphoreType.DMA
    return pl.pallas_call(
        kernel,
        in_specs=[pl.BlockSpec(memory_space=pl.ANY)] * 7,
        out_specs=pl.BlockSpec(memory_space=pltpu.VMEM),
        out_shape=jax.ShapeDtypeStruct((1, 1, D), A_x.dtype),
        scratch_shapes=[
            pltpu.VMEM((1, 1, D), bf),
            pltpu.VMEM((GQ, RQ, H * DH), bf),
            pltpu.VMEM((2, 2, DH, w), bf),
            pltpu.VMEM((GO, RO, D), bf),
            pltpu.VMEM((G3, R3, F), bf),
            pltpu.VMEM((N4, 2, R4, D), bf),
            pltpu.VMEM((2, 8, DH), jnp.float32),
            pltpu.VMEM((H, 8, DH), jnp.float32),
            dma(()),
            dma((RQ // 8,)),
            dma((2, per)),
            dma((NO,)),
            dma((N3,)),
            dma((N4 - 1 + TV,)),
        ],
        compiler_params=pltpu.CompilerParams(
            vmem_limit_bytes=64 * 1024 * 1024,
            disable_bounds_checks=True,
            disable_semaphore_checks=True,
        ),
    )(A_x, kt, vt, A_wq.reshape(GQ, RQ, H * DH), A_wo.reshape(GO, RO, D),
      B_w3.reshape(G3, R3, F), B_w4)
```

```python
import jax
import jax.numpy as jnp
from jax import lax
from jax.experimental import pallas as pl
from jax.experimental.pallas import tpu as pltpu

D = 640
H = 32
DH = 192
F = 1536
EPS = 1e-5
SCALE = DH ** -0.5

LEAD = 26
AHEAD = (32, 32 + LEAD)
KC = 128
NG = 2
GQ, RQ, CQ = 10, 64, 640
GO, RO, NO = 8, 768, 16
G3, R3, N3 = 4, 160, 5
R4, D4 = 128, 32
N4 = F // (2 * R4)
TV = R4 // D4
QC = 2 * DH


def _ln(x):
    m = jnp.mean(x, axis=-1, keepdims=True)
    c = x - m
    v = jnp.mean(c * c, axis=-1, keepdims=True)
    return c / jnp.sqrt(v + EPS)


def _make_kernel(sk, w):
    gw = w // NG
    gn = gw // KC
    per = 2 * NG * gn
    assert max(AHEAD) <= 2 * per - gn
    nt = (((1,), (1,)), ((), ()))

    def kernel(x_hbm, k_hbm, v_hbm, wq_hbm, wo_hbm, w3_hbm, w4_hbm, o_ref,
               xb, wqb, kvb, wob, w3b, w4b, qs, ob,
               sx, sq, skv, so, s3, s4):

        def start(c0, c1):
            for i in range(max(len(c0), len(c1))):
                for p, c in ((0, c0), (1, c1)):
                    if i < len(c):
                        pltpu.make_async_copy(*c[i]).start(priority=p)

        def wait(dst, sem):
            pltpu.make_async_copy(dst, dst, sem).wait()

        def same(hbm, buf, idx, sem):
            return (hbm.at[idx], buf.at[idx], sem)

        def kv_copy(h, i, p):
            kv, c = divmod(i, NG * gn)
            rows = pl.ds(p * (DH // 2), DH // 2)
            return ((k_hbm, v_hbm)[kv].at[h, rows, pl.ds(sk - w + c * KC, KC)],
                    kvb.at[h % 2, kv, rows, pl.ds(c * KC, KC)], skv.at[h % 2, i // gn])

        def wq_copies(r, p):
            return [same(wq_hbm, wqb,
                         (pl.ds(p * (GQ // 2), GQ // 2), pl.ds(8 * r, 8), pl.ds(c, min(CQ, H * DH - c))), sq.at[r])
                    for c in range(0, H * DH, CQ)]

        def wo_pairs(j):
            return [[same(wo_hbm, wob, (pl.ds(4 * p + 2 * g, 2), pl.ds(48 * j + 16 * r, 16), slice(None)), so.at[j])
                     for p in range(2)] for r in range(3) for g in range(2)]

        def w3_pairs(j):
            return [[same(w3_hbm, w3b, (pl.ds(2 * p + g, 1), pl.ds(32 * j + 8 * r, 8), slice(None)), s3.at[j])
                     for p in range(2)] for r in range(4) for g in range(2)]

        def w4_pairs(j, r0, rows, sem):
            return [[(w4_hbm.at[pl.ds((j + N4 * p) * R4 + r, D4), :], w4b.at[j, p, pl.ds(r, D4), :], sem)
                     for p in range(2)] for r in range(r0, r0 + rows, D4)]

        nq = len(wq_copies(0, 0))
        first = [[c for r in range(RQ // 8) for c in wq_copies(r, p)]
                 + [kv_copy(i // per, i % per, p) for i in range(AHEAD[p])] for p in range(2)]
        start([(x_hbm, xb, sx)], first[1][:LEAD])
        start(first[0][:AHEAD[0]], first[1][LEAD:AHEAD[1]])

        wait(xb, sx)
        x = xb[0].astype(jnp.float32)
        xn8 = jnp.broadcast_to(_ln(x), (8, D)).astype(jnp.bfloat16)
        for r in range(RQ // 8):
            wait(wqb.at[:, pl.ds(8 * r, 8), :], sq.at[r])
            start(*[first[p][AHEAD[p] + r * nq:AHEAD[p] + (r + 1) * nq] for p in range(2)])

        tail = ([wo_pairs(j) for j in range(NO)] + [w3_pairs(j) for j in range(N3)]
                + [w4_pairs(j, 0, R4, s4.at[j]) for j in range(N4 - 1)]
                + [w4_pairs(N4 - 1, t * D4, D4, s4.at[N4 - 1 + t]) for t in range(TV)])
        pairs = [pr for g in tail for pr in g]
        cut = len(pairs) - LEAD // 2
        last = [[pr[0] for pr in pairs[:cut]],
                [pr[1] for pr in pairs[:cut]] + [c for pr in pairs[cut:] for c in pr]]

        def head(h, carry):
            slot = h % 2

            @pl.when(slot == 0)
            def _():
                c0 = pl.multiple_of((h // 2) * QC, 128)
                wq2 = wqb[:, :, pl.ds(c0, QC)].reshape(D, QC)
                q2 = jnp.dot(xn8, wq2, preferred_element_type=jnp.float32)
                qs[0] = q2[:, :DH]
                qs[1] = q2[:, DH:]

            q = qs[slot].astype(jnp.bfloat16)

            def arrive(kv, g):
                u = kv * NG + g
                wait(kvb.at[slot, kv, :, pl.ds(g * gw, gw)], skv.at[slot, u])
                nxt = [range(u * gn + AHEAD[p], (u + 1) * gn + AHEAD[p]) for p in range(2)]
                dh = max(r[-1] // per for r in nxt)

                @pl.when(h + dh < H)
                def _():
                    hs = [h + d for d in range(dh + 1)]
                    start(*[[kv_copy(hs[i // per], i % per, p) for i in nxt[p]] for p in range(2)])

                for hh in range(H - dh, H):
                    @pl.when(h == hh)
                    def _():
                        start(*[[kv_copy(hh + i // per, i % per, p) if hh + i // per < H
                                 else last[p][(hh - H) * per + i] for i in nxt[p]] for p in range(2)])
                return kvb[slot, kv, :, g * gw:(g + 1) * gw]

            s = jnp.concatenate(
                [jnp.dot(q, arrive(0, g), preferred_element_type=jnp.float32) * SCALE for g in range(NG)], axis=1)
            p = jnp.exp(s - jnp.max(s, axis=1, keepdims=True))
            l = jnp.sum(p, axis=1, keepdims=True)
            pb = p.astype(jnp.bfloat16)
            o = jnp.zeros((8, DH), jnp.float32)
            for g in range(NG):
                o = o + lax.dot_general(pb[:, g * gw:(g + 1) * gw], arrive(1, g), nt,
                                        preferred_element_type=jnp.float32)
            ob[h] = o / l
            return carry

        lax.fori_loop(0, H, head, 0)

        done = [0]

        def arrive_tail(dst, sem):
            wait(dst, sem)
            a = sum(len(g) for g in tail[:done[0]])
            b = a + len(tail[done[0]])
            start(*[last[p][AHEAD[p] + a:AHEAD[p] + b] for p in range(2)])
            done[0] += 1

        acc = jnp.zeros((8, D), jnp.float32)
        for j in range(NO):
            arrive_tail(wob.at[:, pl.ds(48 * j, 48), :], so.at[j])
            if j % 4 == 3:
                i = j // 4
                for g in range(GO):
                    acc = acc + jnp.dot(ob[4 * g + i].astype(jnp.bfloat16), wob[g, i * DH:(i + 1) * DH, :],
                                        preferred_element_type=jnp.float32)
        hres = x + acc[0:1]
        x1 = _ln(hres)
        y8 = jnp.broadcast_to(_ln(x1), (8, D)).astype(jnp.bfloat16)

        for j in range(N3):
            arrive_tail(w3b.at[:, pl.ds(32 * j, 32), :], s3.at[j])
        t = jnp.dot(y8, w3b[...].reshape(D, F), preferred_element_type=jnp.float32)
        mid = jax.nn.gelu(t, approximate=True).astype(jnp.bfloat16)
        mf = mid.astype(jnp.float32)
        mcol = [jnp.broadcast_to(mf[0:1, (N4 - 1 + N4 * p) * R4:(N4 + N4 * p) * R4], (128, R4)).T
                for p in range(2)]
        acc = jnp.broadcast_to(hres + x1, (8, D))
        for j in range(N4 - 1):
            arrive_tail(w4b.at[j], s4.at[j])
            for p in range(2):
                jj = j + N4 * p
                acc = acc + jnp.dot(mid[:, jj * R4:(jj + 1) * R4], w4b[j, p],
                                    preferred_element_type=jnp.float32)
        accv = jnp.zeros((8, D), jnp.float32)
        for t in range(TV):
            arrive_tail(w4b.at[N4 - 1, :, pl.ds(t * D4, D4), :], s4.at[N4 - 1 + t])
            for p in range(2):
                wv = w4b[N4 - 1, p, t * D4:(t + 1) * D4, :].astype(jnp.float32)
                mc = mcol[p][t * D4:(t + 1) * D4]
                prod = wv * jnp.concatenate([mc] * (D // 128), axis=1)
                accv = accv + jnp.sum(prod.reshape(D4 // 8, 8, D), axis=0)
        out = acc[0:1] + jnp.sum(accv, axis=0, keepdims=True)
        o_ref[0] = out.astype(o_ref.dtype)

    return kernel


@jax.jit
def pallas_sequential_preLN__sliding_block_cached__mixer_s_mlp__decode_kernel(
    A_x: jax.Array,
    A_k_cache: jax.Array,
    A_v_cache: jax.Array,
    A_wq: jax.Array,
    A_wo: jax.Array,
    B_x: jax.Array,
    B_w1: jax.Array,
    B_w2: jax.Array,
    B_w3: jax.Array,
    B_w4: jax.Array,
):
    del B_x, B_w1, B_w2
    assert A_x.shape == (1, 1, D) and A_k_cache.shape[:2] == (1, H) and A_k_cache.shape[3] == DH
    sk = A_k_cache.shape[2]
    w = min(4096, max(256, sk // 4))
    kt = jnp.swapaxes(A_k_cache, 2, 3).reshape(H, DH, sk)
    vt = jnp.swapaxes(A_v_cache, 2, 3).reshape(H, DH, sk)
    bf = jnp.bfloat16
    dma = pltpu.SemaphoreType.DMA
    return pl.pallas_call(
        _make_kernel(sk, w),
        in_specs=[pl.BlockSpec(memory_space=pl.ANY)] * 7,
        out_specs=pl.BlockSpec(memory_space=pltpu.VMEM),
        out_shape=jax.ShapeDtypeStruct((1, 1, D), A_x.dtype),
        scratch_shapes=[
            pltpu.VMEM((1, 1, D), bf),
            pltpu.VMEM((GQ, RQ, H * DH), bf),
            pltpu.VMEM((2, 2, DH, w), bf),
            pltpu.VMEM((GO, RO, D), bf),
            pltpu.VMEM((G3, R3, F), bf),
            pltpu.VMEM((N4, 2, R4, D), bf),
            pltpu.VMEM((2, 8, DH), jnp.float32),
            pltpu.VMEM((H, 8, DH), jnp.float32),
            dma(()),
            dma((RQ // 8,)),
            dma((2, 2 * NG)),
            dma((NO,)),
            dma((N3,)),
            dma((N4 - 1 + TV,)),
        ],
        compiler_params=pltpu.CompilerParams(
            vmem_limit_bytes=64 * 1024 * 1024,
            disable_semaphore_checks=True,
        ),
    )(A_x, kt, vt, A_wq.reshape(GQ, RQ, H * DH), A_wo.reshape(GO, RO, D),
      B_w3.reshape(G3, R3, F), B_w4)
```
